```python
import jax
import jax.numpy as jnp

def _softmax(x, axis=-1):
    return jax.nn.softmax(x, axis=axis)
def _gelu(x):
    return jax.nn.gelu(x, approximate=True)
def _silu(x):
    return jax.nn.silu(x)
def _sigmoid(x):
    return jax.nn.sigmoid(x)
def _layernorm(x, axis=-1, eps=1e-5):
    m = jnp.mean(x, axis=axis, keepdims=True)
    v = jnp.var(x, axis=axis, keepdims=True)
    return (x - m) / jnp.sqrt(v + eps)
def _scatter_add(tgt, idx, src, axis=0):
    return tgt.at[idx].add(src)
def _segment_sum(src, seg, n):
    return jax.ops.segment_sum(src, seg, n)
class _Rng:
    def __init__(self, key):
        self._k = key
    def _next(self):
        self._k, sub = jax.random.split(self._k)
        return sub
    def normal(self, shape):
        return jax.random.normal(self._next(), shape, dtype=jnp.bfloat16)
    def randint(self, lo, hi, shape):
        return jax.random.randint(self._next(), shape, lo, hi, dtype=jnp.int32)
    def uniform(self, shape, lo=0.0, hi=1.0):
        return jax.random.uniform(self._next(), shape, jnp.bfloat16, lo, hi)
    def permutation(self, n):
        return jax.random.permutation(self._next(), n)


kernel_name = 'standalone__groupnorm__prompt'

def setup_inputs():
    _rng = _Rng(jax.random.key(int.from_bytes(__import__("os").urandom(4), "little")))
    _w = (lambda a: (lambda t: t.astype(jnp.bfloat16) if jnp.issubdtype(t.dtype, jnp.floating) else t)(jnp.asarray(a)))
    B = 2
    G = 32
    cpg = max(1, 1024 // G)
    C = G * cpg
    H, W = 32, 2048
    return {
        "x": _w((lambda *s: _rng.normal(s) * 0.05)(B, C, H, W)),
        "g": _w((lambda *s: _rng.normal(s) * 0.05)(C) + 1.0),
        "b": _w((lambda *s: _rng.normal(s) * 0.05)(C)),
    }

def reference(x, g, b):
    G = 32
    B, C, H, W = x.shape[0], x.shape[1], x.shape[2], x.shape[3]
    xr = x.reshape(B, G, C // G, H, W)
    mu = xr.mean(axis=(2, 3, 4), keepdims=True)
    var = ((xr - mu) ** 2).mean(axis=(2, 3, 4), keepdims=True)
    xn = (xr - mu) / jnp.sqrt(var + 1e-5)
    xn = xn.reshape(B, C, H, W)
    return xn * g[None, :, None, None] + b[None, :, None, None]
```

```python
import jax
import jax.numpy as jnp
from jax import lax
import jax.experimental.pallas as pl
import jax.experimental.pallas.tpu as pltpu

_G = 32
_EPS = 1e-5


def _kernel(x_ref, g_ref, b_ref, o_ref, gb_vmem, gb_smem, sem):
    cpg, H, W = x_ref.shape
    C = g_ref.shape[0]
    step = pl.program_id(0)

    @pl.when(step == 0)
    def _():
        gb_vmem[pl.ds(0, C)] = g_ref[...].astype(jnp.float32)
        gb_vmem[pl.ds(C, C)] = b_ref[...].astype(jnp.float32)
        cp = pltpu.make_async_copy(gb_vmem, gb_smem, sem)
        cp.start()
        cp.wait()

    inv_n = 1.0 / (cpg * H * W)

    def fold(v):
        return v.reshape(H // 8, 8, W).sum(axis=0)

    def sum_body(c, acc):
        return acc + fold(x_ref[c].astype(jnp.float32))

    acc = lax.fori_loop(0, cpg, sum_body, jnp.zeros((8, W), jnp.float32))
    mu = jnp.sum(acc, keepdims=True) * inv_n

    def var_body(c, acc):
        d = x_ref[c].astype(jnp.float32) - mu
        return acc + fold(d * d)

    acc = lax.fori_loop(0, cpg, var_body, jnp.zeros((8, W), jnp.float32))
    var = jnp.sum(acc, keepdims=True) * inv_n
    rstd = lax.rsqrt(var + _EPS)

    c0 = (step % _G) * cpg

    def norm_body(c, carry):
        a = rstd * gb_smem[c0 + c]
        d = x_ref[c].astype(jnp.float32) - mu
        o_ref[c] = (d * a + gb_smem[C + c0 + c]).astype(o_ref.dtype)
        return carry

    lax.fori_loop(0, cpg, norm_body, 0)


@jax.jit
def pallas_standalone__groupnorm__prompt_kernel(x, g, b):
    B, C, H, W = x.shape
    cpg = C // _G
    xr = x.reshape(B * C, H, W)
    out = pl.pallas_call(
        _kernel,
        grid=(B * _G,),
        in_specs=[
            pl.BlockSpec((cpg, H, W), lambda i: (i, 0, 0)),
            pl.BlockSpec((C,), lambda i: (0,)),
            pl.BlockSpec((C,), lambda i: (0,)),
        ],
        out_specs=pl.BlockSpec((cpg, H, W), lambda i: (i, 0, 0)),
        out_shape=jax.ShapeDtypeStruct(xr.shape, x.dtype),
        scratch_shapes=[
            pltpu.VMEM((2 * C,), jnp.float32),
            pltpu.SMEM((2 * C,), jnp.float32),
            pltpu.SemaphoreType.DMA(()),
        ],
        compiler_params=pltpu.CompilerParams(
            dimension_semantics=("arbitrary",),
            vmem_limit_bytes=64 * 1024 * 1024,
        ),
    )(xr, g, b)
    return out.reshape(x.shape)
```

```python
import jax
import jax.numpy as jnp
from jax import lax
import jax.experimental.pallas as pl
import jax.experimental.pallas.tpu as pltpu

_G = 32
_EPS = 1e-5
_PHASES = (11, 11, 10)
_WSPLIT = 2
_RTAIL = 2
_WTAIL = 2
_CW = 512
_NACC = 2


def _kernel(x_hbm, g_ref, b_ref, o_hbm, buf, gb_vmem, gb_smem, rsem, rtsem, wsem, wtsem, gsem):
    C = g_ref.shape[0]
    _, NQ, PPQ, NR, _, W = buf.shape
    QPG = NQ // 2
    cpg = QPG * PPQ
    WS = W // _WSPLIT
    nw = PPQ * NR * _WSPLIT

    def rd(pair, slot, h):
        return pltpu.make_async_copy(
            x_hbm.at[pair, pl.ds(h * QPG, QPG)], buf.at[slot, pl.ds(h * QPG, QPG)],
            rsem.at[2 * slot + h])

    def rd_last(pair, slot):
        hd = PPQ - _RTAIL
        return (
            pltpu.make_async_copy(x_hbm.at[pair, pl.ds(QPG, QPG - 1)],
                                  buf.at[slot, pl.ds(QPG, QPG - 1)], rsem.at[2 * slot + 1]),
            pltpu.make_async_copy(x_hbm.at[pair, NQ - 1, pl.ds(0, hd)],
                                  buf.at[slot, NQ - 1, pl.ds(0, hd)], rtsem.at[0]),
            pltpu.make_async_copy(x_hbm.at[pair, NQ - 1, pl.ds(hd, _RTAIL)],
                                  buf.at[slot, NQ - 1, pl.ds(hd, _RTAIL)], rtsem.at[1]),
        )

    def wr(pair, slot, k, sem):
        p = k // (NR * _WSPLIT)
        r = (k // _WSPLIT) % NR
        h = k % _WSPLIT
        return pltpu.make_async_copy(
            buf.at[slot, :, p, r, :, pl.ds(h * WS, WS)],
            o_hbm.at[pair, :, p, r, :, pl.ds(h * WS, WS)], sem)

    def start_reads(pair0, slots, n):
        for s in slots:
            rd(pair0 + s, s, 0).start()
            if s == n - 1:
                for d in rd_last(pair0 + s, s):
                    d.start()
            else:
                rd(pair0 + s, s, 1).start()

    def start_writes(pair, slot, last):
        for k in range(nw):
            sem = wtsem.at[0] if (last and k >= nw - _WTAIL) else wsem.at[slot]
            wr(pair, slot, k, sem).start()

    inv_n = 1.0 / (cpg * NR * 8 * W)
    chunks = [(r, j) for r in range(NR) for j in range(0, W, _CW)]
    ppq_shift = PPQ.bit_length() - 1

    def compute_group(pair, slot, h):
        def idx(c):
            return h * QPG + lax.shift_right_logical(c, ppq_shift), c & (PPQ - 1)

        def ld(q, p, r, j):
            return buf[slot, q, p, r, :, pl.ds(j, _CW)].astype(jnp.float32)

        def total(accs):
            t = accs[0]
            for a in accs[1:]:
                t = t + a
            return jnp.sum(t, keepdims=True)

        zero = tuple(jnp.zeros((8, _CW), jnp.float32) for _ in range(_NACC))

        def sum_body(c, accs):
            q, p = idx(c)
            accs = list(accs)
            for i, (r, j) in enumerate(chunks):
                accs[i % _NACC] = accs[i % _NACC] + ld(q, p, r, j)
            return tuple(accs)

        mu = total(lax.fori_loop(0, cpg, sum_body, zero, unroll=2)) * inv_n
        mu_b = jnp.broadcast_to(mu, (8, _CW))

        def var_body(c, accs):
            q, p = idx(c)
            accs = list(accs)
            for i, (r, j) in enumerate(chunks):
                d = ld(q, p, r, j) - mu_b
                accs[i % _NACC] = accs[i % _NACC] + d * d
            return tuple(accs)

        var = total(lax.fori_loop(0, cpg, var_body, zero, unroll=2)) * inv_n
        rstd = lax.rsqrt(var + _EPS)
        c0 = ((2 * pair + h) & (_G - 1)) * cpg

        def norm_body(c, carry):
            q, p = idx(c)
            a = jnp.broadcast_to(rstd * gb_smem[c0 + c], (8, _CW))
            bb = gb_smem[C + c0 + c]
            for (r, j) in chunks:
                buf[slot, q, p, r, :, pl.ds(j, _CW)] = (
                    (ld(q, p, r, j) - mu_b) * a + bb).astype(buf.dtype)
            return carry

        lax.fori_loop(0, cpg, norm_body, 0, unroll=2)

    start_reads(0, range(_PHASES[0]), _PHASES[0])
    gb_vmem[pl.ds(0, C)] = g_ref[...].astype(jnp.float32)
    gb_vmem[pl.ds(C, C)] = b_ref[...].astype(jnp.float32)
    cp = pltpu.make_async_copy(gb_vmem, gb_smem, gsem)
    cp.start()
    cp.wait()

    pair0 = 0
    for pi, n in enumerate(_PHASES):
        def gbody(j, carry, pair0=pair0):
            s = lax.shift_right_logical(j, 1)
            h = j & 1
            rd(pair0 + s, s, h).wait()
            compute_group(pair0 + s, s, h)
            return carry

        lax.fori_loop(0, 2 * n - 1, gbody, 0)
        head0, head1, tail = rd_last(pair0 + n - 1, n - 1)
        head0.wait()
        head1.wait()
        start_writes(pair0, 0, False)
        tail.wait()
        compute_group(pair0 + n - 1, n - 1, 1)

        def wstart(s, carry, pair0=pair0):
            start_writes(pair0 + s, s, False)
            return carry

        lax.fori_loop(1, n - 1, wstart, 0)
        start_writes(pair0 + n - 1, n - 1, True)

        def wwait(s, carry):
            pltpu.make_async_copy(buf.at[s], buf.at[s], wsem.at[s]).wait()
            return carry

        lax.fori_loop(0, n - 1, wwait, 0)
        for k in range(nw - _WTAIL):
            wr(pair0 + n - 1, n - 1, k, wsem.at[n - 1]).wait()
        nxt = _PHASES[pi + 1] if pi + 1 < len(_PHASES) else 0
        start_reads(pair0 + n, [s for s in range(nxt) if s < n - 1], nxt)
        for k in range(nw - _WTAIL, nw):
            wr(pair0 + n - 1, n - 1, k, wtsem.at[0]).wait()
        start_reads(pair0 + n, [s for s in range(nxt) if s >= n - 1], nxt)
        pair0 += n


@jax.jit
def pallas_standalone__groupnorm__prompt_kernel(x, g, b):
    B, C, H, W = x.shape
    cpg = C // _G
    n_pairs = B * _G // 2
    assert sum(_PHASES) == n_pairs and cpg % 4 == 0 and H % 8 == 0 and W % (128 * _WSPLIT) == 0
    P = max(_PHASES)
    shp = (n_pairs, 8, cpg // 4, H // 8, 8, W)
    out = pl.pallas_call(
        _kernel,
        in_specs=[
            pl.BlockSpec(memory_space=pl.ANY),
            pl.BlockSpec(memory_space=pltpu.VMEM),
            pl.BlockSpec(memory_space=pltpu.VMEM),
        ],
        out_specs=pl.BlockSpec(memory_space=pl.ANY),
        out_shape=jax.ShapeDtypeStruct(shp, x.dtype),
        scratch_shapes=[
            pltpu.VMEM((P,) + shp[1:], x.dtype),
            pltpu.VMEM((2 * C,), jnp.float32),
            pltpu.SMEM((2 * C,), jnp.float32),
            pltpu.SemaphoreType.DMA((2 * P,)),
            pltpu.SemaphoreType.DMA((2,)),
            pltpu.SemaphoreType.DMA((P,)),
            pltpu.SemaphoreType.DMA((1,)),
            pltpu.SemaphoreType.DMA(()),
        ],
        compiler_params=pltpu.CompilerParams(vmem_limit_bytes=(P * 8 + 4) * 1024 * 1024),
    )(x.reshape(shp), g, b)
    return out.reshape(x.shape)
```

```python
import jax
import jax.numpy as jnp
from jax import lax
import jax.experimental.pallas as pl
import jax.experimental.pallas.tpu as pltpu

_G = 32
_EPS = 1e-5
_S = 24
_RPHASES = (24, 20, 20)
_LAG = 2
_DEPTH = _LAG + 2
_WTAIL = 2
_srl = lax.shift_right_logical


def _kernel(x_hbm, g_hbm, b_hbm, o_hbm, buf, g_raw, b_raw, gb_vmem, gb_smem,
            rsem, rtsem, wsem, wtsem, gsem):
    C = g_hbm.shape[0]
    W = buf.shape[-1]
    n_grp = x_hbm.shape[0] // 4
    n_wr = 64

    def rd(gi, s, rest, sem):
        return pltpu.make_async_copy(x_hbm.at[(pl.ds(4 * gi, 4), slice(None)) + rest],
                                     buf.at[(pl.ds(4 * s, 4), slice(None)) + rest], sem)

    def rd_low(gi, s, last):
        parts = [(p, pl.ds(r, 2)) for p in range(2) for r in (0, 2)]
        return [rd(gi, s, rest, rtsem.at[0] if (last and i == 3) else rsem.at[s])
                for i, rest in enumerate(parts)]

    def rd_high(gi, s, o, seg):
        lanes = W // 8
        return rd(gi, s, (2 + _srl(o, 2), o & 3, slice(None), pl.ds(seg * lanes, lanes)), rsem.at[s])

    def wait_group(s):
        blk = buf.at[pl.ds(4 * s, 4)]
        pltpu.make_async_copy(blk, blk, rsem.at[s]).wait()

    def pair_slot(pair):
        return pair % (_S // 2) if isinstance(pair, int) else lax.rem(pair, _S // 2)

    def wr(pair, k, sem=None):
        s2 = pair_slot(pair)
        if isinstance(k, int):
            hf, p, r, off = k >> 5, (k >> 3) & 3, (k >> 1) & 3, (k & 1) * (W // 2)
        else:
            hf, p, r = _srl(k, 5), _srl(k, 3) & 3, _srl(k, 1) & 3
            off = pl.multiple_of((k & 1) * (W // 2), W // 2)
        return pltpu.make_async_copy(
            buf.at[pl.ds(8 * s2, 8), hf, p, r, :, pl.ds(off, W // 2)],
            o_hbm.at[pl.ds(8 * pair, 8), hf, p, r, :, pl.ds(off, W // 2)],
            wsem.at[s2] if sem is None else sem)

    inv_n = 1.0 / (4 * 2 * 4 * 4 * 8 * W)

    def run_slot(t, stats, issue):
        mu2, mu3, rstd3 = stats

        def loc(gi):
            ok = jnp.logical_and(gi >= 0, gi < n_grp)
            return jnp.where(ok, lax.rem(jnp.maximum(gi, 0), _S), _S) * 4, jnp.where(ok, 7, 0)

        locs = loc(t - _LAG), loc(t - _LAG - 1), loc(t - _LAG - 2)
        c0 = ((t - _LAG - 2) & (_G - 1)) * 32

        def body(o, carry):
            acc1, acc2 = carry
            i1, i2, i3 = [(u + _srl(o & m, 1), o & m & 1) for u, m in locs]
            for seg in range(8):
                p, r0 = seg >> 1, (seg & 1) * 2
                issue(o, seg)
                if r0 == 0:
                    scale = rstd3 * gb_smem[c0 + o * 4 + p]
                    shift = gb_smem[C + c0 + o * 4 + p]
                for r in (r0, r0 + 1):
                    acc1 = acc1 + buf[i1[0], i1[1], p, r].astype(jnp.float32)
                    d = buf[i2[0], i2[1], p, r].astype(jnp.float32) - mu2
                    acc2 = acc2 + d * d
                for r in (r0, r0 + 1):
                    d = buf[i3[0], i3[1], p, r].astype(jnp.float32) - mu3
                    buf[i3[0], i3[1], p, r] = (d * scale + shift).astype(buf.dtype)
            return acc1, acc2

        zero = jnp.zeros((8, W), jnp.float32)
        acc1, acc2 = lax.fori_loop(0, 8, body, (zero, zero))
        mu1 = jnp.sum(acc1, keepdims=True) * inv_n
        rstd2 = lax.rsqrt(jnp.sum(acc2, keepdims=True) * inv_n + _EPS)
        return mu1, mu2, rstd2

    for d in rd_low(0, 0, False):
        d.start(priority=1)
    cg = pltpu.make_async_copy(g_hbm, g_raw, gsem.at[0])
    cb = pltpu.make_async_copy(b_hbm, b_raw, gsem.at[1])
    cg.start()
    cb.start()
    buf[4 * _S, 0] = jnp.zeros(buf.shape[2:], buf.dtype)
    cg.wait()
    cb.wait()
    gb_vmem[pl.ds(0, C)] = g_raw[...].astype(jnp.float32)
    gb_vmem[pl.ds(C, C)] = b_raw[...].astype(jnp.float32)
    cp = pltpu.make_async_copy(gb_vmem, gb_smem, gsem.at[0])
    cp.start()
    cp.wait()

    z = jnp.zeros((1, 1), jnp.float32)
    stats = (z, z, z)
    g0 = 0
    w0 = 0
    for pi, n in enumerate(_RPHASES):
        final = pi == len(_RPHASES) - 1
        gend = g0 + n
        s_last = (gend - 1) % _S

        def read_slot(t, stats, g0=g0, gend=gend, s_last=s_last):
            @pl.when(t - _LAG >= g0)
            def _():
                wait_group(lax.rem(t - _LAG, _S))

            @pl.when(t + 1 < gend - 1)
            def _():
                for d in rd_low(t + 1, lax.rem(t + 1, _S), False):
                    d.start(priority=1)

            @pl.when(t + 1 == gend - 1)
            def _():
                for d in rd_low(gend - 1, s_last, True):
                    d.start(priority=1)

            s = lax.rem(t, _S)
            return run_slot(t, stats, lambda o, seg: rd_high(t, s, o, seg).start(priority=0))

        stats = lax.fori_loop(g0, gend, read_slot, stats)
        for gi in range(gend - _LAG, gend - 1):
            wait_group(gi % _S)

        def wait_high(o, c, gend=gend, s_last=s_last):
            for seg in range(8):
                rd_high(gend - 1, s_last, o, seg).wait()
            return c

        lax.fori_loop(0, 8, wait_high, 0)
        low = rd_low(gend - 1, s_last, True)
        for d in low[:3]:
            d.wait()

        wend = n_grp // 2 if final else (gend - _DEPTH) // 2
        for k in range(n_wr):
            wr(w0, k).start()
        low[3].wait()
        wnext = w0 + 1
        if final:
            def drain_slot(t, stats, gend=gend, wnext=wnext):
                def issue(o, seg):
                    if seg & 1 == 0:
                        k = (t - gend) * 32 + o * 4 + (seg >> 1)
                        wr(wnext + _srl(k, 6), k & 63).start()
                return run_slot(t, stats, issue)

            stats = lax.fori_loop(gend, gend + _DEPTH, drain_slot, stats)
            wnext += _DEPTH * 32 // n_wr

        def start_pair(pair, c):
            for k in range(n_wr):
                wr(pair, k).start()
            return c

        lax.fori_loop(wnext, wend - 1, start_pair, 0)
        last = [wr(wend - 1, k, wtsem.at[0] if k >= n_wr - _WTAIL else None) for k in range(n_wr)]
        for d in last:
            d.start()

        def wait_pair(pair, c):
            s2 = pair_slot(pair)
            blk = buf.at[pl.ds(8 * s2, 8)]
            pltpu.make_async_copy(blk, blk, wsem.at[s2]).wait()
            return c

        lax.fori_loop(w0, wend - 1, wait_pair, 0)
        for d in last[:n_wr - _WTAIL]:
            d.wait()
        if not final:
            assert (gend % _S) // 2 != pair_slot(wend - 1)
            for d in rd_low(gend, gend % _S, False):
                d.start(priority=1)
        for d in last[n_wr - _WTAIL:]:
            d.wait()
        g0 = gend
        w0 = wend


@jax.jit
def pallas_standalone__groupnorm__prompt_kernel(x, g, b):
    B, C, H, W = x.shape
    n_grp = B * _G
    assert C == 32 * _G and H == 32 and W % 1024 == 0 and sum(_RPHASES) == n_grp
    shp = (4 * n_grp, 2, 4, 4, 8, W)
    unit_bytes = 2 * 4 * 4 * 8 * W * x.dtype.itemsize
    out = pl.pallas_call(
        _kernel,
        in_specs=[pl.BlockSpec(memory_space=pl.ANY)] * 3,
        out_specs=pl.BlockSpec(memory_space=pl.ANY),
        out_shape=jax.ShapeDtypeStruct(shp, x.dtype),
        scratch_shapes=[
            pltpu.VMEM((4 * _S + 1,) + shp[1:], x.dtype),
            pltpu.VMEM((C,), g.dtype),
            pltpu.VMEM((C,), b.dtype),
            pltpu.VMEM((2 * C,), jnp.float32),
            pltpu.SMEM((2 * C,), jnp.float32),
            pltpu.SemaphoreType.DMA((_S,)),
            pltpu.SemaphoreType.DMA((1,)),
            pltpu.SemaphoreType.DMA((_S // 2,)),
            pltpu.SemaphoreType.DMA((1,)),
            pltpu.SemaphoreType.DMA((2,)),
        ],
        compiler_params=pltpu.CompilerParams(
            vmem_limit_bytes=(4 * _S + 1) * unit_bytes + 8 * 1024 * 1024),
    )(x.reshape(shp), g, b)
    return out.reshape(x.shape)
```

```python
import jax
import jax.numpy as jnp
from jax import lax
import jax.experimental.pallas as pl
import jax.experimental.pallas.tpu as pltpu

_G = 32
_EPS = 1e-5
_S = 24
_RPHASES = (24, 20, 20)
_LAG = 2
_DEPTH = _LAG + 2
_RTAIL = 2
_WTAIL = 2
_srl = lax.shift_right_logical


def _kernel(x_hbm, g_hbm, b_hbm, o_hbm, buf, g_raw, b_raw, gb_vmem, gb_smem,
            rsem, wsem, wtsem, gsem):
    C = g_hbm.shape[0]
    W = buf.shape[-1]
    n_grp = x_hbm.shape[0] // 4
    n_wr = 64

    def rd(gi, s, rest, sem):
        return pltpu.make_async_copy(x_hbm.at[(pl.ds(4 * gi, 4), slice(None)) + rest],
                                     buf.at[(pl.ds(4 * s, 4), slice(None)) + rest], sem)

    def rd_low(gi, s, o, j, sem):
        p, r = (o >> 2, o & 3) if isinstance(o, int) else (_srl(o, 2), o & 3)
        return rd(gi, s, (p, r, slice(None), pl.ds(j * (W // 2), W // 2)), sem)

    def start_low_all(gi):
        for o in range(8):
            for j in range(2):
                rd_low(gi, gi % _S, o, j, rsem.at[gi % _S]).start(priority=1)

    def rd_high(gi, s, o, seg):
        lanes = W // 8
        return rd(gi, s, (2 + _srl(o, 2), o & 3, slice(None), pl.ds(seg * lanes, lanes)), rsem.at[s])

    def wait_group(s):
        blk = buf.at[pl.ds(4 * s, 4)]
        pltpu.make_async_copy(blk, blk, rsem.at[s]).wait()

    def pair_slot(pair):
        return pair % (_S // 2) if isinstance(pair, int) else lax.rem(pair, _S // 2)

    def wr(pair, k, sem=None):
        s2 = pair_slot(pair)
        if isinstance(k, int):
            hf, p, r, off = k >> 5, (k >> 3) & 3, (k >> 1) & 3, (k & 1) * (W // 2)
        else:
            hf, p, r = _srl(k, 5), _srl(k, 3) & 3, _srl(k, 1) & 3
            off = pl.multiple_of((k & 1) * (W // 2), W // 2)
        return pltpu.make_async_copy(
            buf.at[pl.ds(8 * s2, 8), hf, p, r, :, pl.ds(off, W // 2)],
            o_hbm.at[pl.ds(8 * pair, 8), hf, p, r, :, pl.ds(off, W // 2)],
            wsem.at[s2] if sem is None else sem)

    inv_n = 1.0 / (4 * 2 * 4 * 4 * 8 * W)

    def run_slot(t, stats, issue):
        mu2, mu3, rstd3 = stats

        def loc(gi):
            ok = jnp.logical_and(gi >= 0, gi < n_grp)
            return jnp.where(ok, lax.rem(jnp.maximum(gi, 0), _S), _S) * 4, jnp.where(ok, 7, 0)

        locs = loc(t - _LAG), loc(t - _LAG - 1), loc(t - _LAG - 2)
        c0 = ((t - _LAG - 2) & (_G - 1)) * 32

        def body(o, carry):
            acc1, acc2 = carry
            i1, i2, i3 = [(u + _srl(o & m, 1), o & m & 1) for u, m in locs]
            for seg in range(8):
                p, r0 = seg >> 1, (seg & 1) * 2
                issue(o, seg)
                if r0 == 0:
                    scale = rstd3 * gb_smem[c0 + o * 4 + p]
                    shift = gb_smem[C + c0 + o * 4 + p]
                for r in (r0, r0 + 1):
                    acc1 = acc1 + buf[i1[0], i1[1], p, r].astype(jnp.float32)
                    d = buf[i2[0], i2[1], p, r].astype(jnp.float32) - mu2
                    acc2 = acc2 + d * d
                for r in (r0, r0 + 1):
                    d = buf[i3[0], i3[1], p, r].astype(jnp.float32) - mu3
                    buf[i3[0], i3[1], p, r] = (d * scale + shift).astype(buf.dtype)
            return acc1, acc2

        zero = jnp.zeros((8, W), jnp.float32)
        acc1, acc2 = lax.fori_loop(0, 8, body, (zero, zero))
        mu1 = jnp.sum(acc1, keepdims=True) * inv_n
        rstd2 = lax.rsqrt(jnp.sum(acc2, keepdims=True) * inv_n + _EPS)
        return mu1, mu2, rstd2

    cg = pltpu.make_async_copy(g_hbm, g_raw, gsem.at[0])
    cb = pltpu.make_async_copy(b_hbm, b_raw, gsem.at[1])
    cg.start()
    cb.start()
    start_low_all(0)
    buf[4 * _S, 0] = jnp.zeros(buf.shape[2:], buf.dtype)
    cg.wait()
    cb.wait()
    gb_vmem[pl.ds(0, C)] = g_raw[...].astype(jnp.float32)
    gb_vmem[pl.ds(C, C)] = b_raw[...].astype(jnp.float32)
    cp = pltpu.make_async_copy(gb_vmem, gb_smem, gsem.at[0])
    cp.start()
    cp.wait()

    z = jnp.zeros((1, 1), jnp.float32)
    stats = (z, z, z)
    g0 = 0
    w0 = 0
    for pi, n in enumerate(_RPHASES):
        final = pi == len(_RPHASES) - 1
        gend = g0 + n
        s_last = (gend - 1) % _S

        def read_slot(t, stats, g0=g0, pos="mid"):
            @pl.when(t - _LAG >= g0)
            def _():
                wait_group(lax.rem(t - _LAG, _S))

            s = lax.rem(t, _S)

            def issue(o, seg):
                rd_high(t, s, o, seg).start(priority=0)
                if pos != "first" and seg & 3 == 1:
                    si = jnp.where(o >= 8 - _RTAIL, _S, s) if pos == "last" else s
                    rd_low(t, s, o, seg >> 2, rsem.at[si]).start(priority=1)

            return run_slot(t, stats, issue)

        stats = read_slot(jnp.int32(g0), stats, pos="first")
        stats = lax.fori_loop(g0 + 1, gend - 1, read_slot, stats)
        stats = read_slot(jnp.int32(gend - 1), stats, pos="last")
        for gi in range(gend - _LAG, gend - 1):
            wait_group(gi % _S)

        def wait_high(o, c, gend=gend, s_last=s_last):
            for seg in range(8):
                rd_high(gend - 1, s_last, o, seg).wait()
            return c

        lax.fori_loop(0, 8, wait_high, 0)
        for o in range(8 - _RTAIL):
            for j in range(2):
                rd_low(gend - 1, s_last, o, j, rsem.at[s_last]).wait()

        wend = n_grp // 2 if final else (gend - _DEPTH) // 2
        for k in range(n_wr):
            wr(w0, k).start()
        for o in range(8 - _RTAIL, 8):
            for j in range(2):
                rd_low(gend - 1, s_last, o, j, rsem.at[_S]).wait()
        wnext = w0 + 1
        if final:
            def drain_slot(t, stats, gend=gend, wnext=wnext):
                def issue(o, seg):
                    if seg & 1 == 0:
                        k = (t - gend) * 32 + o * 4 + (seg >> 1)
                        wr(wnext + _srl(k, 6), k & 63).start()
                return run_slot(t, stats, issue)

            stats = lax.fori_loop(gend, gend + _DEPTH, drain_slot, stats)
            wnext += _DEPTH * 32 // n_wr

        def start_pair(pair, c):
            for k in range(n_wr):
                wr(pair, k).start()
            return c

        lax.fori_loop(wnext, wend - 1, start_pair, 0)
        last = [wr(wend - 1, k, wtsem.at[0] if k >= n_wr - _WTAIL else None) for k in range(n_wr)]
        for d in last:
            d.start()

        def wait_pair(pair, c):
            s2 = pair_slot(pair)
            blk = buf.at[pl.ds(8 * s2, 8)]
            pltpu.make_async_copy(blk, blk, wsem.at[s2]).wait()
            return c

        lax.fori_loop(w0, wend - 1, wait_pair, 0)
        for d in last[:n_wr - _WTAIL]:
            d.wait()
        if not final:
            assert (gend % _S) // 2 != pair_slot(wend - 1)
            start_low_all(gend)
        for d in last[n_wr - _WTAIL:]:
            d.wait()
        g0 = gend
        w0 = wend


@jax.jit
def pallas_standalone__groupnorm__prompt_kernel(x, g, b):
    B, C, H, W = x.shape
    n_grp = B * _G
    assert C == 32 * _G and H == 32 and W % 1024 == 0 and sum(_RPHASES) == n_grp
    shp = (4 * n_grp, 2, 4, 4, 8, W)
    unit_bytes = 2 * 4 * 4 * 8 * W * x.dtype.itemsize
    out = pl.pallas_call(
        _kernel,
        in_specs=[pl.BlockSpec(memory_space=pl.ANY)] * 3,
        out_specs=pl.BlockSpec(memory_space=pl.ANY),
        out_shape=jax.ShapeDtypeStruct(shp, x.dtype),
        scratch_shapes=[
            pltpu.VMEM((4 * _S + 1,) + shp[1:], x.dtype),
            pltpu.VMEM((C,), g.dtype),
            pltpu.VMEM((C,), b.dtype),
            pltpu.VMEM((2 * C,), jnp.float32),
            pltpu.SMEM((2 * C,), jnp.float32),
            pltpu.SemaphoreType.DMA((_S + 1,)),
            pltpu.SemaphoreType.DMA((_S // 2,)),
            pltpu.SemaphoreType.DMA((1,)),
            pltpu.SemaphoreType.DMA((2,)),
        ],
        compiler_params=pltpu.CompilerParams(
            vmem_limit_bytes=(4 * _S + 1) * unit_bytes + 8 * 1024 * 1024),
    )(x.reshape(shp), g, b)
    return out.reshape(x.shape)
```

```python
import jax
import jax.numpy as jnp
from jax import lax
import jax.experimental.pallas as pl
import jax.experimental.pallas.tpu as pltpu

_G = 32
_EPS = 1e-5
_S = 28
_RPHASES = (26, 19, 19)
_LAG = 2
_DEPTH = _LAG + 2
_WNS = 7
_WTAIL = 2
_A = 13
_WA = 0
_CT = 16
_srl = lax.shift_right_logical

_LOW = [(_A + 32 * j, 32) for j in range(4)]
_HIGH = [(_A + 128 + 16 * j, 16) for j in range(6)] + [(_A + 224, 32 - _A), (0, _A)]
_WRITE = [(hf, st, n) for hf in range(2)
          for st, n in [(0, _WA)] + [(_WA + 8 * i, min(8, 256 - _WA - 8 * i)) for i in range(32)]
          if n > 0]


def _write_blocks(n_units):
    blocks, u = [], 0
    while n_units - u >= 2 * _WNS or n_units - u == _WNS:
        blocks.append((u, _WNS))
        u += _WNS
    if u < n_units:
        h = (n_units - u + 1) // 2
        blocks += [(u, h), (u + h, n_units - u - h)]
    return blocks


def _kernel(x_hbm, g_hbm, b_hbm, o_hbm, buf, g_raw, b_raw, gb_vmem, gb_smem,
            rsem, wsem, wtsem, gsem):
    C = g_hbm.shape[0]
    n_units = x_hbm.shape[0]
    n_grp = n_units // 4
    ring = 4 * _S
    n_wsem = wsem.shape[0]
    blocks = _write_blocks(n_units)
    n_reg = sum(1 for _, sz in blocks if sz == _WNS)
    assert all(u0 % ring + sz <= ring for u0, sz in blocks)

    def rd_low(gi, s, i, last=False):
        tiles = pl.ds(*_LOW[i])
        sem = rsem.at[_S if (last and i == len(_LOW) - 1) else s]
        return pltpu.make_async_copy(x_hbm.at[pl.ds(4 * gi, 4), :, tiles],
                                     buf.at[pl.ds(4 * s, 4), :, tiles], sem)

    def start_low(gi, s, last=False):
        for i in range(len(_LOW)):
            rd_low(gi, s, i, last).start(priority=1)

    def rd_high(gi, s, o, seg):
        q = (o + seg) & 7
        u, hf, tiles = _srl(q, 1), q & 1, pl.ds(*_HIGH[seg])
        return pltpu.make_async_copy(x_hbm.at[4 * gi + u, hf, tiles],
                                     buf.at[4 * s + u, hf, tiles], rsem.at[s])

    def wait_group(s):
        blk = buf.at[pl.ds(4 * s, 4)]
        pltpu.make_async_copy(blk, blk, rsem.at[s]).wait()

    def block_geom(bi):
        if isinstance(bi, int):
            u0, sz = blocks[bi]
            return u0, sz, u0 % ring, bi % n_wsem
        return bi * _WNS, _WNS, lax.rem(bi * _WNS, ring), lax.rem(bi, n_wsem)

    def wr(bi, part, sem=None):
        u0, sz, v0, si = block_geom(bi)
        hf, tiles = part[0], pl.ds(part[1], part[2])
        return pltpu.make_async_copy(buf.at[pl.ds(v0, sz), hf, tiles],
                                     o_hbm.at[pl.ds(u0, sz), hf, tiles],
                                     wsem.at[si] if sem is None else sem)

    def start_block(bi, c=0):
        for part in _WRITE:
            wr(bi, part).start()
        return c

    def wait_block(bi, c=0):
        _, sz, v0, si = block_geom(bi)
        blk = buf.at[pl.ds(v0, sz)]
        pltpu.make_async_copy(blk, blk, wsem.at[si]).wait()
        return c

    inv_n = 1.0 / (4 * 2 * 256 * 8 * 128)

    def run_slot(t, stats, issue):
        mu2, mu3, rstd3 = stats

        def loc(gi):
            ok = jnp.logical_and(gi >= 0, gi < n_grp)
            return jnp.where(ok, lax.rem(jnp.maximum(gi, 0), _S), _S) * 4, jnp.where(ok, 7, 0)

        locs = loc(t - _LAG), loc(t - _LAG - 1), loc(t - _LAG - 2)
        c0 = ((t - _LAG - 2) & (_G - 1)) * 32

        def body(o, carry):
            acc1, acc2 = carry
            i1, i2, i3 = [(u + _srl(o & m, 1), o & m & 1) for u, m in locs]
            for seg in range(8):
                issue(o, seg)
                if seg & 1 == 0:
                    ch = c0 + o * 4 + (seg >> 1)
                    scale = rstd3 * gb_smem[ch]
                    shift = gb_smem[C + ch]
                chunks = [pl.ds(t0, _CT) for t0 in range(seg * 32, seg * 32 + 32, _CT)]
                for tiles in chunks:
                    acc1 = acc1 + buf[i1[0], i1[1], tiles].astype(jnp.float32)
                    d = buf[i2[0], i2[1], tiles].astype(jnp.float32) - mu2
                    acc2 = acc2 + d * d
                for tiles in chunks:
                    d = buf[i3[0], i3[1], tiles].astype(jnp.float32) - mu3
                    buf[i3[0], i3[1], tiles] = (d * scale + shift).astype(buf.dtype)
            return acc1, acc2

        zero = jnp.zeros((_CT, 8, 128), jnp.float32)
        acc1, acc2 = lax.fori_loop(0, 8, body, (zero, zero))
        mu1 = jnp.sum(jnp.sum(acc1, axis=0), keepdims=True) * inv_n
        var2 = jnp.sum(jnp.sum(acc2, axis=0), keepdims=True) * inv_n
        return mu1, mu2, lax.rsqrt(var2 + _EPS)

    cg = pltpu.make_async_copy(g_hbm, g_raw, gsem.at[0])
    cb = pltpu.make_async_copy(b_hbm, b_raw, gsem.at[1])
    cg.start()
    cb.start()
    start_low(0, 0)
    buf[ring, 0] = jnp.zeros(buf.shape[2:], buf.dtype)
    cg.wait()
    cb.wait()
    gb_vmem[pl.ds(0, C)] = g_raw[...].astype(jnp.float32)
    gb_vmem[pl.ds(C, C)] = b_raw[...].astype(jnp.float32)
    cp = pltpu.make_async_copy(gb_vmem, gb_smem, gsem.at[0])
    cp.start()
    cp.wait()

    z = jnp.zeros((1, 1), jnp.float32)
    stats = (z, z, z)
    g0 = 0
    w0 = 0
    for pi, n in enumerate(_RPHASES):
        final = pi == len(_RPHASES) - 1
        gend = g0 + n
        s_last = (gend - 1) % _S
        assert 4 * (gend - _S) <= blocks[w0][0]

        def read_slot(t, stats, g0=g0, gend=gend, s_last=s_last):
            @pl.when(t - _LAG >= g0)
            def _():
                wait_group(lax.rem(t - _LAG, _S))

            @pl.when(t + 1 < gend - 1)
            def _():
                start_low(t + 1, lax.rem(t + 1, _S))

            @pl.when(t + 1 == gend - 1)
            def _():
                start_low(gend - 1, s_last, last=True)

            s = lax.rem(t, _S)
            return run_slot(t, stats, lambda o, seg: rd_high(t, s, o, seg).start(priority=0))

        stats = lax.fori_loop(g0, gend, read_slot, stats)
        for gi in range(gend - _LAG, gend - 1):
            wait_group(gi % _S)

        def wait_high(o, c, gend=gend, s_last=s_last):
            for seg in range(8):
                rd_high(gend - 1, s_last, o, seg).wait()
            return c

        lax.fori_loop(0, 8, wait_high, 0)
        for i in range(len(_LOW) - 1):
            rd_low(gend - 1, s_last, i, last=True).wait()

        done_units = n_units if final else 4 * (gend - _DEPTH)
        wend = sum(1 for u0, sz in blocks if u0 + sz <= done_units)
        assert wend - w0 <= n_wsem
        start_block(w0)
        rd_low(gend - 1, s_last, len(_LOW) - 1, last=True).wait()
        wnext = w0 + 1
        if final:
            def drain_slot(t, stats, gend=gend, wnext=wnext):
                stats = run_slot(t, stats, lambda o, seg: None)
                start_block(wnext + (t - gend))
                return stats

            stats = lax.fori_loop(gend, gend + _DEPTH, drain_slot, stats)
            wnext += _DEPTH
            assert blocks[wnext][0] <= 4 * (gend - _DEPTH)

        reg_end = min(wend - 1, n_reg)
        lax.fori_loop(wnext, reg_end, start_block, 0)
        for bi in range(reg_end, wend - 1):
            start_block(bi)
        n_head = len(_WRITE) - _WTAIL
        last = [wr(wend - 1, part, None if k < n_head else wtsem.at[0])
                for k, part in enumerate(_WRITE)]
        for d in last:
            d.start()
        lax.fori_loop(w0, reg_end, wait_block, 0)
        for bi in range(reg_end, wend - 1):
            wait_block(bi)
        for d in last[:n_head]:
            d.wait()
        if not final:
            assert 4 * (gend + 1 - _S) <= blocks[wend - 1][0]
            start_low(gend, gend % _S)
        for d in last[n_head:]:
            d.wait()
        g0 = gend
        w0 = wend


@jax.jit
def pallas_standalone__groupnorm__prompt_kernel(x, g, b):
    B, C, H, W = x.shape
    n_grp = B * _G
    assert C == 32 * _G and H * W == 64 * 1024 and H % 8 == 0 and W % 128 == 0
    assert sum(_RPHASES) == n_grp
    shp = (4 * n_grp, 2, 256, 8, 128)
    strips = B * C * H // 8
    xt = x.reshape(strips, 8, W // 128, 128).transpose(0, 2, 1, 3).reshape(shp)
    unit_bytes = 2 * 256 * 8 * 128 * x.dtype.itemsize
    out = pl.pallas_call(
        _kernel,
        in_specs=[pl.BlockSpec(memory_space=pl.ANY)] * 3,
        out_specs=pl.BlockSpec(memory_space=pl.ANY),
        out_shape=jax.ShapeDtypeStruct(shp, x.dtype),
        scratch_shapes=[
            pltpu.VMEM((4 * _S + 1,) + shp[1:], x.dtype),
            pltpu.VMEM((C,), g.dtype),
            pltpu.VMEM((C,), b.dtype),
            pltpu.VMEM((2 * C,), jnp.float32),
            pltpu.SMEM((2 * C,), jnp.float32),
            pltpu.SemaphoreType.DMA((_S + 1,)),
            pltpu.SemaphoreType.DMA((4 * _S // _WNS + 1,)),
            pltpu.SemaphoreType.DMA((1,)),
            pltpu.SemaphoreType.DMA((2,)),
        ],
        compiler_params=pltpu.CompilerParams(
            vmem_limit_bytes=(4 * _S + 1) * unit_bytes + 8 * 1024 * 1024),
    )(xt, g, b)
    return out.reshape(strips, W // 128, 8, 128).transpose(0, 2, 1, 3).reshape(x.shape)
```

```python
import jax
import jax.numpy as jnp
from jax import lax
import jax.experimental.pallas as pl
import jax.experimental.pallas.tpu as pltpu

_G = 32
_EPS = 1e-5
_S = 28
_RPHASES = (26, 19, 19)
_LAG = 2
_DEPTH = _LAG + 2
_WNS = 7
_WTAIL = 2
_A = 13
_WA = 4
_WP = 8
_CLEAN = 0
_PACE = 50
_CT = 16
_srl = lax.shift_right_logical

_LOW = [(_A + 32 * j, 32) for j in range(4)]
_HIGH = [(_A + 128 + 16 * j, 16) for j in range(6)] + [(_A + 224, 32 - _A), (0, _A)]
_WRITE = [(hf, st, n) for hf in range(2)
          for st, n in [(0, _WA)] + [(t0, min(_WP, 256 - t0)) for t0 in range(_WA, 256, _WP)]
          if n > 0]


def _write_blocks(n_units):
    blocks, u = [], 0
    while n_units - u >= 2 * _WNS or n_units - u == _WNS:
        blocks.append((u, _WNS))
        u += _WNS
    if u < n_units:
        h = (n_units - u + 1) // 2
        blocks += [(u, h), (u + h, n_units - u - h)]
    return blocks


def _kernel(x_hbm, g_hbm, b_hbm, o_hbm, buf, g_raw, b_raw, gb_vmem, gb_smem,
            pace, rsem, wsem):
    C = g_hbm.shape[0]
    n_units = x_hbm.shape[0]
    n_grp = n_units // 4
    ring = 4 * _S
    blocks = _write_blocks(n_units)
    n_reg = sum(1 for _, sz in blocks if sz == _WNS)
    assert all(u0 % ring + sz <= ring for u0, sz in blocks)

    n_low_last = len(_LOW) - _CLEAN

    def rd_low(gi, s, i, last=False):
        tiles = pl.ds(*_LOW[i])
        sem = wsem.at[3] if (last and i == n_low_last - 1) else rsem.at[gi & 3]
        return pltpu.make_async_copy(x_hbm.at[pl.ds(4 * gi, 4), :, tiles],
                                     buf.at[pl.ds(4 * s, 4), :, tiles], sem)

    def start_low(gi, s, last=False):
        for i in range(n_low_last if last else len(_LOW)):
            rd_low(gi, s, i, last).start(priority=1)

    def rd_clean(gi, s, k):
        q, tiles = k & 7, pl.ds(_LOW[n_low_last][0] + _srl(k, 3) * 16, 16)
        return pltpu.make_async_copy(x_hbm.at[4 * gi + _srl(q, 1), q & 1, tiles],
                                     buf.at[4 * s + _srl(q, 1), q & 1, tiles], rsem.at[gi & 3])

    def rd_high(gi, s, o, seg):
        q = (o + seg) & 7
        u, hf, tiles = _srl(q, 1), q & 1, pl.ds(*_HIGH[seg])
        return pltpu.make_async_copy(x_hbm.at[4 * gi + u, hf, tiles],
                                     buf.at[4 * s + u, hf, tiles], rsem.at[gi & 3])

    def wait_all(v0, n, sem):
        blk = buf.at[pl.ds(v0, n)]
        pltpu.make_async_copy(blk, blk, sem).wait()

    def wr(bi, part, wrap, si=None):
        u0, sz = blocks[bi] if isinstance(bi, int) else (bi * _WNS, _WNS)
        if isinstance(bi, int):
            after = int(u0 >= wrap)
        else:
            after = (u0 >= wrap).astype(jnp.int32)
        v0 = u0 - wrap + ring * (1 - after)
        hf, tiles = part[0], pl.ds(part[1], part[2])
        return pltpu.make_async_copy(buf.at[pl.ds(v0, sz), hf, tiles],
                                     o_hbm.at[pl.ds(u0, sz), hf, tiles],
                                     wsem.at[after if si is None else si])

    inv_n = 1.0 / (4 * 2 * 256 * 8 * 128)

    def run_slot(t, stats, issue):
        mu2, mu3, rstd3 = stats

        def loc(gi):
            ok = jnp.logical_and(gi >= 0, gi < n_grp)
            return jnp.where(ok, lax.rem(jnp.maximum(gi, 0), _S), _S) * 4, jnp.where(ok, 7, 0)

        locs = loc(t - _LAG), loc(t - _LAG - 1), loc(t - _LAG - 2)
        c0 = ((t - _LAG - 2) & (_G - 1)) * 32

        def body(o, carry):
            acc1, acc2 = carry
            i1, i2, i3 = [(u + _srl(o & m, 1), o & m & 1) for u, m in locs]
            for seg in range(8):
                issue(o, seg)
                if seg & 1 == 0:
                    ch = c0 + o * 4 + (seg >> 1)
                    scale = rstd3 * gb_smem[ch]
                    shift = gb_smem[C + ch]
                chunks = [pl.ds(t0, _CT) for t0 in range(seg * 32, seg * 32 + 32, _CT)]
                for tiles in chunks:
                    acc1 = acc1 + buf[i1[0], i1[1], tiles].astype(jnp.float32)
                    d = buf[i2[0], i2[1], tiles].astype(jnp.float32) - mu2
                    acc2 = acc2 + d * d
                for tiles in chunks:
                    d = buf[i3[0], i3[1], tiles].astype(jnp.float32) - mu3
                    buf[i3[0], i3[1], tiles] = (d * scale + shift).astype(buf.dtype)
            return acc1, acc2

        zero = jnp.zeros((_CT, 8, 128), jnp.float32)
        acc1, acc2 = lax.fori_loop(0, 8, body, (zero, zero))
        mu1 = jnp.sum(jnp.sum(acc1, axis=0), keepdims=True) * inv_n
        var2 = jnp.sum(jnp.sum(acc2, axis=0), keepdims=True) * inv_n
        return mu1, mu2, lax.rsqrt(var2 + _EPS)

    cg = pltpu.make_async_copy(g_hbm, g_raw, wsem.at[0])
    cb = pltpu.make_async_copy(b_hbm, b_raw, wsem.at[1])
    cg.start()
    cb.start()
    start_low(0, 0)
    buf[ring, 0] = jnp.zeros(buf.shape[2:], buf.dtype)
    pace[0] = 0
    cg.wait()
    cb.wait()
    gb_vmem[pl.ds(0, C)] = g_raw[...].astype(jnp.float32)
    gb_vmem[pl.ds(C, C)] = b_raw[...].astype(jnp.float32)
    cp = pltpu.make_async_copy(gb_vmem, gb_smem, wsem.at[0])
    cp.start()
    cp.wait()

    z = jnp.zeros((1, 1), jnp.float32)
    stats = (z, z, z)
    g0 = 0
    w0 = 0
    for pi, n in enumerate(_RPHASES):
        final = pi == len(_RPHASES) - 1
        gend = g0 + n
        s_last = (gend - 1) % _S
        assert 4 * (gend - _S) <= blocks[w0][0]

        def read_slot(t, stats, g0=g0, gend=gend, s_last=s_last):
            @pl.when(t - _LAG >= g0)
            def _():
                wait_all(4 * lax.rem(t - _LAG, _S), 4, rsem.at[(t - _LAG) & 3])

            @pl.when(t + 1 < gend - 1)
            def _():
                start_low(t + 1, lax.rem(t + 1, _S))

            @pl.when(t + 1 == gend - 1)
            def _():
                start_low(gend - 1, s_last, last=True)

            s = lax.rem(t, _S)
            return run_slot(t, stats, lambda o, seg: rd_high(t, s, o, seg).start(priority=0))

        stats = lax.fori_loop(g0, gend, read_slot, stats)

        def clean(k, zero, gend=gend, s_last=s_last):
            rd_clean(gend - 1, s_last, k + zero).start(priority=0)
            for _ in range(_PACE):
                zero = (zero << 1) ^ zero
            return zero

        if _CLEAN:
            pace[0] = lax.fori_loop(0, 16 * _CLEAN, clean, pace[0])
        for gi in range(gend - _LAG, gend - 1):
            wait_all(4 * (gi % _S), 4, rsem.at[gi & 3])

        def wait_high(o, c, gend=gend, s_last=s_last):
            for seg in range(8):
                rd_high(gend - 1, s_last, o, seg).wait()
            for j in range(2 * _CLEAN):
                rd_clean(gend - 1, s_last, j * 8 + o).wait()
            return c

        lax.fori_loop(0, 8, wait_high, 0)
        for i in range(n_low_last - 1):
            rd_low(gend - 1, s_last, i, last=True).wait()

        done_units = n_units if final else 4 * (gend - _DEPTH)
        wend = sum(1 for u0, sz in blocks if u0 + sz <= done_units)
        u_first, u_last = blocks[w0][0], blocks[wend - 1][0]
        wrap = (u_first // ring + 1) * ring

        def start_block(bi, c=0, wrap=wrap):
            for part in _WRITE:
                wr(bi, part, wrap).start()
            return c

        start_block(w0)
        rd_low(gend - 1, s_last, n_low_last - 1, last=True).wait()
        wnext = w0 + 1
        if final:
            def drain_slot(t, stats, gend=gend, wnext=wnext):
                stats = run_slot(t, stats, lambda o, seg: None)
                start_block(wnext + (t - gend))
                return stats

            stats = lax.fori_loop(gend, gend + _DEPTH, drain_slot, stats)
            wnext += _DEPTH
            assert blocks[wnext][0] <= 4 * (gend - _DEPTH)

        reg_end = min(wend - 1, n_reg)
        lax.fori_loop(wnext, reg_end, start_block, 0)
        for bi in range(reg_end, wend - 1):
            start_block(bi)
        n_head = len(_WRITE) - _WTAIL
        last = [wr(wend - 1, part, wrap, 2 if k < n_head else 3) for k, part in enumerate(_WRITE)]
        for d in last:
            d.start()
        wait_all(u_first % ring, min(u_last, wrap) - u_first, wsem.at[0])
        if u_last > wrap:
            wait_all(0, u_last - wrap, wsem.at[1])
        for d in last[:n_head]:
            d.wait()
        if not final:
            assert 4 * (gend + 1 - _S) <= u_last
            start_low(gend, gend % _S)
        for d in last[n_head:]:
            d.wait()
        g0 = gend
        w0 = wend


@jax.jit
def pallas_standalone__groupnorm__prompt_kernel(x, g, b):
    B, C, H, W = x.shape
    n_grp = B * _G
    assert C == 32 * _G and H * W == 64 * 1024 and H % 8 == 0 and W % 128 == 0
    assert sum(_RPHASES) == n_grp
    shp = (4 * n_grp, 2, 256, 8, 128)
    strips = B * C * H // 8
    xt = x.reshape(strips, 8, W // 128, 128).transpose(0, 2, 1, 3).reshape(shp)
    unit_bytes = 2 * 256 * 8 * 128 * x.dtype.itemsize
    out = pl.pallas_call(
        _kernel,
        in_specs=[pl.BlockSpec(memory_space=pl.ANY)] * 3,
        out_specs=pl.BlockSpec(memory_space=pl.ANY),
        out_shape=jax.ShapeDtypeStruct(shp, x.dtype),
        scratch_shapes=[
            pltpu.VMEM((4 * _S + 1,) + shp[1:], x.dtype),
            pltpu.VMEM((C,), g.dtype),
            pltpu.VMEM((C,), b.dtype),
            pltpu.VMEM((2 * C,), jnp.float32),
            pltpu.SMEM((2 * C,), jnp.float32),
            pltpu.SMEM((1,), jnp.int32),
            pltpu.SemaphoreType.DMA((4,)),
            pltpu.SemaphoreType.DMA((4,)),
        ],
        compiler_params=pltpu.CompilerParams(
            vmem_limit_bytes=(4 * _S + 1) * unit_bytes + 8 * 1024 * 1024),
    )(xt, g, b)
    return out.reshape(strips, W // 128, 8, 128).transpose(0, 2, 1, 3).reshape(x.shape)
```

```python
import jax
import jax.numpy as jnp
from jax import lax
import jax.experimental.pallas as pl
import jax.experimental.pallas.tpu as pltpu

_G = 32
_EPS = 1e-5
_S = 28
_GEND = (26, 45, 64)
_LAG = 2
_DEPTH = _LAG + 2
_WNS = 7
_WTAIL = 2
_A = 13
_WA = 0
_CLEAN = 1
_PACE = 60
_CT = 16
_srl = lax.shift_right_logical

_LOW = [(_A + 32 * j, 32) for j in range(4)]
_HIGH = [(_A + 128 + 16 * j, 16) for j in range(6)] + [(_A + 224, 32 - _A), (0, _A)]


def _write_blocks(n_units):
    blocks, u = [], 0
    while n_units - u >= 2 * _WNS or n_units - u == _WNS:
        blocks.append((u, _WNS))
        u += _WNS
    if u < n_units:
        h = (n_units - u + 1) // 2
        blocks += [(u, h), (u + h, n_units - u - h)]
    return blocks


def _any_eq(t, values):
    hit = t == values[0]
    for v in values[1:]:
        hit = jnp.logical_or(hit, t == v)
    return hit


def _kernel(x_hbm, g_hbm, b_hbm, o_hbm, buf, g_raw, b_raw, gb_vmem, gb_smem, pace, rsem, wsem):
    C = g_hbm.shape[0]
    n_units = x_hbm.shape[0]
    n_grp = n_units // 4
    ring = 4 * _S
    blocks = _write_blocks(n_units)
    n_reg = sum(1 for _, sz in blocks if sz == _WNS)
    assert all(u0 % ring + sz <= ring for u0, sz in blocks)
    n_low_last = len(_LOW) - _CLEAN

    def slot_of(gi):
        return gi % _S if isinstance(gi, int) else lax.rem(gi, _S)

    def rd_low(gi, i, last=False):
        tiles = pl.ds(*_LOW[i])
        sem = wsem.at[3] if (last and i == n_low_last - 1) else rsem.at[gi & 3]
        return pltpu.make_async_copy(x_hbm.at[pl.ds(4 * gi, 4), :, tiles],
                                     buf.at[pl.ds(4 * slot_of(gi), 4), :, tiles], sem)

    def start_low(gi, last=False):
        for i in range(n_low_last if last else len(_LOW)):
            rd_low(gi, i, last).start(priority=1)

    def rd_piece(gi, s, q, tiles):
        return pltpu.make_async_copy(x_hbm.at[4 * gi + _srl(q, 1), q & 1, tiles],
                                     buf.at[4 * s + _srl(q, 1), q & 1, tiles], rsem.at[gi & 3])

    def rd_high(gi, s, o, seg):
        return rd_piece(gi, s, (o + seg) & 7, pl.ds(*_HIGH[seg]))

    def rd_clean(gi, s, k):
        return rd_piece(gi, s, k & 7, pl.ds(_LOW[n_low_last][0] + _srl(k, 3) * 16, 16))

    def wait_all(v0, n, sem):
        blk = buf.at[pl.ds(v0, n)]
        pltpu.make_async_copy(blk, blk, sem).wait()

    def block_copies(bi, wrap, fn, last=False):
        if isinstance(bi, int):
            u0, sz = blocks[bi]
            after = int(u0 >= wrap)
        else:
            u0, sz = bi * _WNS, _WNS
            after = (u0 >= wrap).astype(jnp.int32)
        v0 = u0 - wrap + ring * (1 - after)

        def piece(hf, t0, n, tail=False):
            sem = wsem.at[(3 if tail else 2) if last else after]
            fn(pltpu.make_async_copy(buf.at[pl.ds(v0, sz), hf, pl.ds(t0, n)],
                                     o_hbm.at[pl.ds(u0, sz), hf, pl.ds(t0, n)], sem), tail)

        def regular(hf, lo, hi):
            def body(i, c):
                piece(hf, _WA + 8 * i, 8)
                return c
            lax.fori_loop(lo, hi, body, 0)

        for hf in range(2):
            n_tail = _WTAIL if (last and hf == 1) else 0
            if _WA:
                piece(hf, 0, _WA)
            regular(hf, 0, 32 - max(n_tail, 1))
            for i in range(32 - max(n_tail, 1), 32):
                piece(hf, _WA + 8 * i, min(8, 256 - _WA - 8 * i), tail=n_tail > 0)

    def start_block(bi, wrap, last=False):
        block_copies(bi, wrap, lambda d, tail: d.start(), last)

    inv_n = 1.0 / (4 * 2 * 256 * 8 * 128)

    def run_slot(t, stats, issue, segs):
        mu2, mu3, rstd3 = stats

        def loc(gi):
            ok = jnp.logical_and(gi >= 0, gi < n_grp)
            return jnp.where(ok, lax.rem(jnp.maximum(gi, 0), _S), _S) * 4, jnp.where(ok, 7, 0)

        locs = loc(t - _LAG), loc(t - _LAG - 1), loc(t - _LAG - 2)
        c0 = ((t - _LAG - 2) & (_G - 1)) * 32

        def body(it, carry):
            acc1, acc2 = carry
            o, seg0 = (it, 0) if segs == 8 else (_srl(it * segs, 3), (it * segs) & 7)
            i1, i2, i3 = [(u + _srl(o & m, 1), o & m & 1) for u, m in locs]
            for j in range(segs):
                if issue is not None:
                    issue(o, j)
                if j & 1 == 0:
                    ch = c0 + it * (segs // 2) + (j >> 1)
                    scale = rstd3 * gb_smem[ch]
                    shift = gb_smem[C + ch]
                chunks = [pl.ds(seg0 * 32 + t0, _CT) for t0 in range(j * 32, j * 32 + 32, _CT)]
                for tiles in chunks:
                    acc1 = acc1 + buf[i1[0], i1[1], tiles].astype(jnp.float32)
                    d = buf[i2[0], i2[1], tiles].astype(jnp.float32) - mu2
                    acc2 = acc2 + d * d
                for tiles in chunks:
                    d = buf[i3[0], i3[1], tiles].astype(jnp.float32) - mu3
                    buf[i3[0], i3[1], tiles] = (d * scale + shift).astype(buf.dtype)
            return acc1, acc2

        zero = jnp.zeros((_CT, 8, 128), jnp.float32)
        acc1, acc2 = lax.fori_loop(0, 64 // segs, body, (zero, zero))
        mu1 = jnp.sum(jnp.sum(acc1, axis=0), keepdims=True) * inv_n
        var2 = jnp.sum(jnp.sum(acc2, axis=0), keepdims=True) * inv_n
        return mu1, mu2, lax.rsqrt(var2 + _EPS)

    def finish_reads(t):
        s = slot_of(t)

        def clean(k, zero):
            rd_clean(t, s, k + zero).start(priority=0)
            for _ in range(_PACE):
                zero = (zero << 1) ^ zero
            return zero

        if _CLEAN:
            pace[0] = lax.fori_loop(0, 16 * _CLEAN, clean, pace[0])
        for d in range(_LAG - 1, 0, -1):
            wait_all(4 * slot_of(t - d), 4, rsem.at[(t - d) & 3])

        def wait_high(o, c):
            for seg in range(8):
                rd_high(t, s, o, seg).wait()
            for j in range(2 * _CLEAN):
                rd_clean(t, s, j * 8 + o).wait()
            return c

        lax.fori_loop(0, 8, wait_high, 0)
        for i in range(n_low_last - 1):
            rd_low(t, i, last=True).wait()

    done_units = [4 * (ge - _DEPTH) for ge in _GEND[:-1]] + [n_units]
    wend = [sum(1 for u0, sz in blocks if u0 + sz <= du) for du in done_units]

    def write_phase(p, stats=None):
        w0, w1, gend = (wend[p - 1] if p else 0), wend[p], _GEND[p]
        final = p == len(_GEND) - 1
        u_first, u_last = blocks[w0][0], blocks[w1 - 1][0]
        wrap = (u_first // ring + 1) * ring
        start_block(w0, wrap)
        rd_low(gend - 1, n_low_last - 1, last=True).wait()
        wnext = w0 + 1
        if final:
            def drain_slot(t, stats):
                stats = run_slot(t, stats, None, 2)
                start_block(w0 + 1 + (t - gend), wrap)
                return stats

            lax.fori_loop(gend, gend + _DEPTH, drain_slot, stats)
            wnext += _DEPTH
            assert blocks[wnext][0] <= 4 * (gend - _DEPTH)

        def start_regular(bi, c):
            start_block(bi, wrap)
            return c

        reg_end = min(w1 - 1, n_reg)
        lax.fori_loop(wnext, reg_end, start_regular, 0)
        for bi in range(reg_end, w1 - 1):
            start_block(bi, wrap)
        start_block(w1 - 1, wrap, last=True)
        wait_all(u_first % ring, min(u_last, wrap) - u_first, wsem.at[0])
        if u_last > wrap:
            wait_all(0, u_last - wrap, wsem.at[1])
        tails = []
        block_copies(w1 - 1, wrap, lambda d, tail: tails.append(d) if tail else d.wait(), True)
        if not final:
            assert 4 * (gend + 1 - _S) <= u_last and 4 * (_GEND[p + 1] - _S) <= blocks[w1][0]
            start_low(gend)
        for d in tails:
            d.wait()

    cg = pltpu.make_async_copy(g_hbm, g_raw, wsem.at[0])
    cb = pltpu.make_async_copy(b_hbm, b_raw, wsem.at[1])
    cg.start()
    cb.start()
    start_low(0)

    def clear(i, c):
        buf[ring, 0, pl.ds(i * _CT, _CT)] = jnp.zeros((_CT, 8, 128), buf.dtype)
        return c

    lax.fori_loop(0, 256 // _CT, clear, 0)
    pace[0] = 0
    cg.wait()
    cb.wait()
    gb_vmem[pl.ds(0, C)] = g_raw[...].astype(jnp.float32)
    gb_vmem[pl.ds(C, C)] = b_raw[...].astype(jnp.float32)
    cp = pltpu.make_async_copy(gb_vmem, gb_smem, wsem.at[0])
    cp.start()
    cp.wait()

    firsts = (0,) + _GEND[:-1]
    lasts = tuple(ge - 1 for ge in _GEND)

    def time_slot(t, stats):
        @pl.when(jnp.logical_not(_any_eq(t, [f + d for f in firsts for d in range(_LAG)])))
        def _():
            wait_all(4 * lax.rem(t - _LAG, _S), 4, rsem.at[(t - _LAG) & 3])

        next_is_last = _any_eq(t + 1, lasts)
        is_last = _any_eq(t, lasts)

        @pl.when(jnp.logical_not(jnp.logical_or(next_is_last, is_last)))
        def _():
            start_low(t + 1)

        @pl.when(next_is_last)
        def _():
            start_low(t + 1, last=True)

        s = lax.rem(t, _S)
        stats = run_slot(t, stats, lambda o, seg: rd_high(t, s, o, seg).start(priority=0), 8)

        @pl.when(is_last)
        def _():
            finish_reads(t)

        for p in range(len(_GEND) - 1):
            @pl.when(t == lasts[p])
            def _():
                write_phase(p)

        return stats

    z = jnp.zeros((1, 1), jnp.float32)
    stats = lax.fori_loop(0, n_grp, time_slot, (z, z, z))
    write_phase(len(_GEND) - 1, stats)


@jax.jit
def pallas_standalone__groupnorm__prompt_kernel(x, g, b):
    B, C, H, W = x.shape
    n_grp = B * _G
    assert C == 32 * _G and H * W == 64 * 1024 and H % 8 == 0 and W % 128 == 0
    assert _GEND[-1] == n_grp
    shp = (4 * n_grp, 2, 256, 8, 128)
    strips = B * C * H // 8
    xt = x.reshape(strips, 8, W // 128, 128).transpose(0, 2, 1, 3).reshape(shp)
    unit_bytes = 2 * 256 * 8 * 128 * x.dtype.itemsize
    out = pl.pallas_call(
        _kernel,
        in_specs=[pl.BlockSpec(memory_space=pl.ANY)] * 3,
        out_specs=pl.BlockSpec(memory_space=pl.ANY),
        out_shape=jax.ShapeDtypeStruct(shp, x.dtype),
        scratch_shapes=[
            pltpu.VMEM((4 * _S + 1,) + shp[1:], x.dtype),
            pltpu.VMEM((C,), g.dtype),
            pltpu.VMEM((C,), b.dtype),
            pltpu.VMEM((2 * C,), jnp.float32),
            pltpu.SMEM((2 * C,), jnp.float32),
            pltpu.SMEM((1,), jnp.int32),
            pltpu.SemaphoreType.DMA((4,)),
            pltpu.SemaphoreType.DMA((4,)),
        ],
        compiler_params=pltpu.CompilerParams(
            vmem_limit_bytes=(4 * _S + 1) * unit_bytes + 8 * 1024 * 1024),
    )(xt, g, b)
    return out.reshape(strips, W // 128, 8, 128).transpose(0, 2, 1, 3).reshape(x.shape)
```

```python
import jax
import jax.numpy as jnp
from jax import lax
import jax.experimental.pallas as pl
import jax.experimental.pallas.tpu as pltpu

_G = 32
_EPS = 1e-5
_S = 28
_GEND = (26, 45, 64)
_LAG = 2
_DEPTH = _LAG + 2
_WNS = 7
_A = 13
_WA = 7
_CLEAN = 1
_PACE = 50
_CT = 16
_srl = lax.shift_right_logical

_LOW = [(_A + 32 * j, 32) for j in range(4)]
_HIGH = [(_A + 128 + 16 * j, 16) for j in range(6)] + [(_A + 224, 32 - _A), (0, _A)]


def _write_blocks(n_units):
    blocks, u = [], 0
    while n_units - u >= 2 * _WNS or n_units - u == _WNS:
        blocks.append((u, _WNS))
        u += _WNS
    if u < n_units:
        h = (n_units - u + 1) // 2
        blocks += [(u, h), (u + h, n_units - u - h)]
    return blocks


def _any_eq(t, values):
    hit = t == values[0]
    for v in values[1:]:
        hit = jnp.logical_or(hit, t == v)
    return hit


def _kernel(x_hbm, g_hbm, b_hbm, o_hbm, buf, g_raw, b_raw, gb_vmem, gb_smem, pace, rsem, wsem):
    C = g_hbm.shape[0]
    n_units = x_hbm.shape[0]
    n_grp = n_units // 4
    ring = 4 * _S
    blocks = _write_blocks(n_units)
    n_reg = sum(1 for _, sz in blocks if sz == _WNS)
    assert all(u0 % ring + sz <= ring for u0, sz in blocks)
    n_low_last = len(_LOW) - _CLEAN

    def slot_of(gi):
        return gi % _S if isinstance(gi, int) else lax.rem(gi, _S)

    def rd_low(gi, i, last=False):
        tiles = pl.ds(*_LOW[i])
        sem = wsem.at[2] if (last and i == n_low_last - 1) else rsem.at[gi & 3]
        return pltpu.make_async_copy(x_hbm.at[pl.ds(4 * gi, 4), :, tiles],
                                     buf.at[pl.ds(4 * slot_of(gi), 4), :, tiles], sem)

    def start_low(gi, last=False):
        for i in range(n_low_last if last else len(_LOW)):
            rd_low(gi, i, last).start(priority=1)

    def rd_piece(gi, s, q, tiles):
        return pltpu.make_async_copy(x_hbm.at[4 * gi + _srl(q, 1), q & 1, tiles],
                                     buf.at[4 * s + _srl(q, 1), q & 1, tiles], rsem.at[gi & 3])

    def rd_high(gi, s, o, seg):
        return rd_piece(gi, s, (o + seg) & 7, pl.ds(*_HIGH[seg]))

    def rd_clean(gi, s, k):
        return rd_piece(gi, s, k & 7, pl.ds(_LOW[n_low_last][0] + _srl(k, 3) * 16, 16))

    def wait_all(v0, n, sem):
        blk = buf.at[pl.ds(v0, n)]
        pltpu.make_async_copy(blk, blk, sem).wait()

    def wait_group(gi):
        wait_all(4 * slot_of(gi), 4, rsem.at[gi & 3])

    def start_block(bi, wrap):
        if isinstance(bi, int):
            u0, sz = blocks[bi]
            after = int(u0 >= wrap)
        else:
            u0, sz = bi * _WNS, _WNS
            after = (u0 >= wrap).astype(jnp.int32)
        v0 = u0 - wrap + ring * (1 - after)

        def piece(hf, t0, n):
            pltpu.make_async_copy(buf.at[pl.ds(v0, sz), hf, pl.ds(t0, n)],
                                  o_hbm.at[pl.ds(u0, sz), hf, pl.ds(t0, n)], wsem.at[after]).start()

        for hf in range(2):
            def regular(i, c):
                piece(hf, _WA + 8 * i, 8)
                return c

            if _WA:
                piece(hf, 0, _WA)
            lax.fori_loop(0, 31 if _WA else 32, regular, 0)
            if _WA:
                piece(hf, _WA + 248, 8 - _WA)

    inv_n = 1.0 / (4 * 2 * 256 * 8 * 128)

    def run_slot(t, stats, issue, segs):
        mu2, mu3, rstd3 = stats

        def loc(gi):
            ok = jnp.logical_and(gi >= 0, gi < n_grp)
            return jnp.where(ok, lax.rem(jnp.maximum(gi, 0), _S), _S) * 4, jnp.where(ok, 7, 0)

        locs = loc(t - _LAG), loc(t - _LAG - 1), loc(t - _LAG - 2)
        c0 = ((t - _LAG - 2) & (_G - 1)) * 32

        def body(it, carry):
            acc1, acc2 = carry
            o, seg0 = (it, 0) if segs == 8 else (_srl(it * segs, 3), (it * segs) & 7)
            i1, i2, i3 = [(u + _srl(o & m, 1), o & m & 1) for u, m in locs]
            for j in range(segs):
                if issue is not None:
                    issue(o, j)
                if j & 1 == 0:
                    ch = c0 + it * (segs // 2) + (j >> 1)
                    scale = rstd3 * gb_smem[ch]
                    shift = gb_smem[C + ch]
                chunks = [pl.ds(seg0 * 32 + t0, _CT) for t0 in range(j * 32, j * 32 + 32, _CT)]
                for tiles in chunks:
                    acc1 = acc1 + buf[i1[0], i1[1], tiles].astype(jnp.float32)
                    d = buf[i2[0], i2[1], tiles].astype(jnp.float32) - mu2
                    acc2 = acc2 + d * d
                for tiles in chunks:
                    d = buf[i3[0], i3[1], tiles].astype(jnp.float32) - mu3
                    buf[i3[0], i3[1], tiles] = (d * scale + shift).astype(buf.dtype)
            return acc1, acc2

        zero = jnp.zeros((_CT, 8, 128), jnp.float32)
        acc1, acc2 = lax.fori_loop(0, 64 // segs, body, (zero, zero))
        mu1 = jnp.sum(jnp.sum(acc1, axis=0), keepdims=True) * inv_n
        var2 = jnp.sum(jnp.sum(acc2, axis=0), keepdims=True) * inv_n
        return mu1, mu2, lax.rsqrt(var2 + _EPS)

    def finish_reads(t):
        s = slot_of(t)

        def clean(k, zero):
            rd_clean(t, s, k + zero).start(priority=0)
            for _ in range(_PACE):
                zero = (zero << 1) ^ zero
            return zero

        pace[0] = lax.fori_loop(0, 16 * _CLEAN, clean, pace[0])
        for d in range(_LAG - 1, 0, -1):
            wait_group(t - d)

        def wait_high(o, c):
            for seg in range(8):
                rd_high(t, s, o, seg).wait()
            for j in range(2 * _CLEAN):
                rd_clean(t, s, j * 8 + o).wait()
            return c

        lax.fori_loop(0, 8, wait_high, 0)
        for i in range(n_low_last - 1):
            rd_low(t, i, last=True).wait()

    done_units = [4 * (ge - _DEPTH) for ge in _GEND[:-1]] + [n_units]
    wend = [sum(1 for u0, sz in blocks if u0 + sz <= du) for du in done_units]

    def write_phase(p, stats=None):
        w0, w1, gend = (wend[p - 1] if p else 0), wend[p], _GEND[p]
        final = p == len(_GEND) - 1
        u_first, u_end = blocks[w0][0], sum(blocks[w1 - 1])
        wrap = (u_first // ring + 1) * ring
        start_block(w0, wrap)
        rd_low(gend - 1, n_low_last - 1, last=True).wait()
        wnext = w0 + 1
        if final:
            def drain_slot(t, stats):
                stats = run_slot(t, stats, None, 2)
                start_block(w0 + 1 + (t - gend), wrap)
                return stats

            lax.fori_loop(gend, gend + _DEPTH, drain_slot, stats)
            wnext += _DEPTH
            assert blocks[wnext][0] <= 4 * (gend - _DEPTH)

        def start_regular(bi, c):
            start_block(bi, wrap)
            return c

        lax.fori_loop(wnext, min(w1, n_reg), start_regular, 0)
        for bi in range(n_reg, w1):
            start_block(bi, wrap)
        wait_all(u_first % ring, min(u_end, wrap) - u_first, wsem.at[0])
        if u_end > wrap:
            wait_all(0, u_end - wrap, wsem.at[1])
        if not final:
            assert 4 * (_GEND[p + 1] - _S) <= u_end
            start_low(gend)

    cg = pltpu.make_async_copy(g_hbm, g_raw, wsem.at[0])
    cb = pltpu.make_async_copy(b_hbm, b_raw, wsem.at[1])
    cg.start()
    cb.start()
    start_low(0)

    def clear(i, c):
        buf[ring, 0, pl.ds(i * _CT, _CT)] = jnp.zeros((_CT, 8, 128), buf.dtype)
        return c

    lax.fori_loop(0, 256 // _CT, clear, 0)
    pace[0] = 0
    cg.wait()
    cb.wait()
    gb_vmem[pl.ds(0, C)] = g_raw[...].astype(jnp.float32)
    gb_vmem[pl.ds(C, C)] = b_raw[...].astype(jnp.float32)
    cp = pltpu.make_async_copy(gb_vmem, gb_smem, wsem.at[0])
    cp.start()
    cp.wait()

    firsts = (0,) + _GEND[:-1]
    lasts = tuple(ge - 1 for ge in _GEND)

    def time_slot(t, stats):
        @pl.when(jnp.logical_not(_any_eq(t, [f + d for f in firsts for d in range(_LAG)])))
        def _():
            wait_group(t - _LAG)

        next_is_last = _any_eq(t + 1, lasts)
        is_last = _any_eq(t, lasts)

        @pl.when(jnp.logical_not(jnp.logical_or(next_is_last, is_last)))
        def _():
            start_low(t + 1)

        @pl.when(next_is_last)
        def _():
            start_low(t + 1, last=True)

        s = lax.rem(t, _S)
        stats = run_slot(t, stats, lambda o, seg: rd_high(t, s, o, seg).start(priority=0), 8)

        @pl.when(is_last)
        def _():
            finish_reads(t)

        for p in range(len(_GEND) - 1):
            @pl.when(t == lasts[p])
            def _():
                write_phase(p)

        return stats

    z = jnp.zeros((1, 1), jnp.float32)
    stats = lax.fori_loop(0, n_grp, time_slot, (z, z, z))
    write_phase(len(_GEND) - 1, stats)


@jax.jit
def pallas_standalone__groupnorm__prompt_kernel(x, g, b):
    B, C, H, W = x.shape
    n_grp = B * _G
    assert C == 32 * _G and H * W == 64 * 1024 and H % 8 == 0 and W % 128 == 0
    assert _GEND[-1] == n_grp
    shp = (4 * n_grp, 2, 256, 8, 128)
    strips = B * C * H // 8
    xt = x.reshape(strips, 8, W // 128, 128).transpose(0, 2, 1, 3).reshape(shp)
    unit_bytes = 2 * 256 * 8 * 128 * x.dtype.itemsize
    out = pl.pallas_call(
        _kernel,
        in_specs=[pl.BlockSpec(memory_space=pl.ANY)] * 3,
        out_specs=pl.BlockSpec(memory_space=pl.ANY),
        out_shape=jax.ShapeDtypeStruct(shp, x.dtype),
        scratch_shapes=[
            pltpu.VMEM((4 * _S + 1,) + shp[1:], x.dtype),
            pltpu.VMEM((C,), g.dtype),
            pltpu.VMEM((C,), b.dtype),
            pltpu.VMEM((2 * C,), jnp.float32),
            pltpu.SMEM((2 * C,), jnp.float32),
            pltpu.SMEM((1,), jnp.int32),
            pltpu.SemaphoreType.DMA((4,)),
            pltpu.SemaphoreType.DMA((3,)),
        ],
        compiler_params=pltpu.CompilerParams(
            vmem_limit_bytes=(4 * _S + 1) * unit_bytes + 8 * 1024 * 1024),
    )(xt, g, b)
    return out.reshape(strips, W // 128, 8, 128).transpose(0, 2, 1, 3).reshape(x.shape)
```

```python
import jax
import jax.numpy as jnp
from jax import lax
import jax.experimental.pallas as pl
import jax.experimental.pallas.tpu as pltpu

_G = 32
_EPS = 1e-5
_S = 28
_GEND = (26, 45, 64)
_LAG = 2
_DEPTH = _LAG + 2
_WNS = 7
_A = 13
_WA = 0
_CT = 16
_srl = lax.shift_right_logical

_FRONT_LOW = [(_A + 32 * j, 32) for j in range(4)]
_BACK_LOW = [(_A + 128 + 32 * j, 32) for j in range(3)] + [(_A + 224, 32 - _A), (0, _A)]
_HIGH_SIZE = [16] * 6 + [32 - _A, _A]
_FRONT_HIGH = [_A + 16 * j for j in range(7)] + [128]
_BACK_HIGH = [_A + 128 + 16 * j for j in range(7)] + [0]


def _write_blocks(n_units):
    blocks, u = [], 0
    while n_units - u >= 2 * _WNS or n_units - u == _WNS:
        blocks.append((u, _WNS))
        u += _WNS
    if u < n_units:
        h = (n_units - u + 1) // 2
        blocks += [(u, h), (u + h, n_units - u - h)]
    return blocks


def _any_eq(t, values):
    hit = t == values[0]
    for v in values[1:]:
        hit = jnp.logical_or(hit, t == v)
    return hit


def _kernel(x_hbm, g_hbm, b_hbm, o_hbm, buf, g_raw, b_raw, gb_vmem, gb_smem, rsem, wsem):
    C = g_hbm.shape[0]
    n_units = x_hbm.shape[0]
    n_grp = n_units // 4
    ring = 4 * _S
    blocks = _write_blocks(n_units)
    n_reg = sum(1 for _, sz in blocks if sz == _WNS)
    assert all(u0 % ring + sz <= ring for u0, sz in blocks)

    def slot_of(gi):
        return gi % _S if isinstance(gi, int) else lax.rem(gi, _S)

    def start_low(gi, pieces):
        for first, n in pieces:
            tiles = pl.ds(first, n)
            pltpu.make_async_copy(x_hbm.at[pl.ds(4 * gi, 4), :, tiles],
                                  buf.at[pl.ds(4 * slot_of(gi), 4), :, tiles],
                                  rsem.at[gi & 3]).start(priority=1)

    def wait_all(v0, n, sem):
        blk = buf.at[pl.ds(v0, n)]
        pltpu.make_async_copy(blk, blk, sem).wait()

    def wait_group(gi):
        wait_all(4 * slot_of(gi), 4, rsem.at[gi & 3])

    def start_block(bi, wrap):
        if isinstance(bi, int):
            u0, sz = blocks[bi]
            after = int(u0 >= wrap)
        else:
            u0, sz = bi * _WNS, _WNS
            after = (u0 >= wrap).astype(jnp.int32)
        v0 = u0 - wrap + ring * (1 - after)

        def piece(hf, t0, n):
            pltpu.make_async_copy(buf.at[pl.ds(v0, sz), hf, pl.ds(t0, n)],
                                  o_hbm.at[pl.ds(u0, sz), hf, pl.ds(t0, n)], wsem.at[after]).start()

        for hf in range(2):
            def regular(i, c):
                piece(hf, _WA + 8 * i, 8)
                return c

            if _WA:
                piece(hf, 0, _WA)
            lax.fori_loop(0, 31 if _WA else 32, regular, 0)
            if _WA:
                piece(hf, _WA + 248, 8 - _WA)

    inv_n = 1.0 / (4 * 2 * 256 * 8 * 128)

    def run_slot(t, stats, issue, segs):
        mu2, mu3, rstd3 = stats

        def loc(gi):
            ok = jnp.logical_and(gi >= 0, gi < n_grp)
            return jnp.where(ok, lax.rem(jnp.maximum(gi, 0), _S), _S) * 4, jnp.where(ok, 7, 0)

        locs = loc(t - _LAG), loc(t - _LAG - 1), loc(t - _LAG - 2)
        c0 = ((t - _LAG - 2) & (_G - 1)) * 32

        def body(it, carry):
            acc1, acc2 = carry
            o, seg0 = (it, 0) if segs == 8 else (_srl(it * segs, 3), (it * segs) & 7)
            i1, i2, i3 = [(u + _srl(o & m, 1), o & m & 1) for u, m in locs]
            for j in range(segs):
                if issue is not None:
                    issue(o, j)
                if j & 1 == 0:
                    ch = c0 + it * (segs // 2) + (j >> 1)
                    scale = rstd3 * gb_smem[ch]
                    shift = gb_smem[C + ch]
                chunks = [pl.ds(seg0 * 32 + t0, _CT) for t0 in range(j * 32, j * 32 + 32, _CT)]
                for tiles in chunks:
                    acc1 = acc1 + buf[i1[0], i1[1], tiles].astype(jnp.float32)
                    d = buf[i2[0], i2[1], tiles].astype(jnp.float32) - mu2
                    acc2 = acc2 + d * d
                for tiles in chunks:
                    d = buf[i3[0], i3[1], tiles].astype(jnp.float32) - mu3
                    buf[i3[0], i3[1], tiles] = (d * scale + shift).astype(buf.dtype)
            return acc1, acc2

        zero = jnp.zeros((_CT, 8, 128), jnp.float32)
        acc1, acc2 = lax.fori_loop(0, 64 // segs, body, (zero, zero))
        mu1 = jnp.sum(jnp.sum(acc1, axis=0), keepdims=True) * inv_n
        var2 = jnp.sum(jnp.sum(acc2, axis=0), keepdims=True) * inv_n
        return mu1, mu2, lax.rsqrt(var2 + _EPS)

    done_units = [4 * (ge - _DEPTH) for ge in _GEND[:-1]] + [n_units]
    wend = [sum(1 for u0, sz in blocks if u0 + sz <= du) for du in done_units]

    def write_phase(p, stats=None):
        w0, w1, gend = (wend[p - 1] if p else 0), wend[p], _GEND[p]
        final = p == len(_GEND) - 1
        u_first, u_end = blocks[w0][0], sum(blocks[w1 - 1])
        wrap = (u_first // ring + 1) * ring
        start_block(w0, wrap)
        for gi in range(gend - _LAG, gend):
            wait_group(gi)
        wnext = w0 + 1
        if final:
            def drain_slot(t, stats):
                stats = run_slot(t, stats, None, 2)
                start_block(w0 + 1 + (t - gend), wrap)
                return stats

            lax.fori_loop(gend, gend + _DEPTH, drain_slot, stats)
            wnext += _DEPTH
            assert blocks[wnext][0] <= 4 * (gend - _DEPTH)

        def start_regular(bi, c):
            start_block(bi, wrap)
            return c

        lax.fori_loop(wnext, min(w1, n_reg), start_regular, 0)
        for bi in range(n_reg, w1):
            start_block(bi, wrap)
        wait_all(u_first % ring, min(u_end, wrap) - u_first, wsem.at[0])
        if u_end > wrap:
            wait_all(0, u_end - wrap, wsem.at[1])
        if not final:
            assert 4 * (_GEND[p + 1] - _S) <= u_end
            start_low(gend, _FRONT_LOW + _BACK_LOW)

    cg = pltpu.make_async_copy(g_hbm, g_raw, wsem.at[0])
    cb = pltpu.make_async_copy(b_hbm, b_raw, wsem.at[1])
    cg.start()
    cb.start()
    start_low(0, _FRONT_LOW + _BACK_LOW)

    def clear(i, c):
        buf[ring, 0, pl.ds(i * _CT, _CT)] = jnp.zeros((_CT, 8, 128), buf.dtype)
        return c

    lax.fori_loop(0, 256 // _CT, clear, 0)
    cg.wait()
    cb.wait()
    gb_vmem[pl.ds(0, C)] = g_raw[...].astype(jnp.float32)
    gb_vmem[pl.ds(C, C)] = b_raw[...].astype(jnp.float32)
    cp = pltpu.make_async_copy(gb_vmem, gb_smem, wsem.at[0])
    cp.start()
    cp.wait()

    firsts = (0,) + _GEND[:-1]
    lasts = tuple(ge - 1 for ge in _GEND)

    def time_slot(t, stats):
        @pl.when(jnp.logical_not(_any_eq(t, [f + d for f in firsts for d in range(_LAG)])))
        def _():
            wait_group(t - _LAG)

        is_last = _any_eq(t, lasts)

        @pl.when(jnp.logical_not(jnp.logical_or(_any_eq(t, firsts), is_last)))
        def _():
            start_low(t, _FRONT_LOW)

        gh = jnp.where(is_last, t, t + 1)
        sh = lax.rem(gh, _S)
        first_tile = [jnp.where(is_last, f, bk) for f, bk in zip(_FRONT_HIGH, _BACK_HIGH)]

        def start_high(o, seg):
            q = (o + seg) & 7
            u, hf, tiles = _srl(q, 1), q & 1, pl.ds(first_tile[seg], _HIGH_SIZE[seg])
            pltpu.make_async_copy(x_hbm.at[4 * gh + u, hf, tiles], buf.at[4 * sh + u, hf, tiles],
                                  rsem.at[gh & 3]).start(priority=0)

        stats = run_slot(t, stats, start_high, 8)

        for p in range(len(_GEND) - 1):
            @pl.when(t == lasts[p])
            def _():
                write_phase(p)

        return stats

    z = jnp.zeros((1, 1), jnp.float32)
    stats = lax.fori_loop(0, n_grp, time_slot, (z, z, z))
    write_phase(len(_GEND) - 1, stats)


@jax.jit
def pallas_standalone__groupnorm__prompt_kernel(x, g, b):
    B, C, H, W = x.shape
    n_grp = B * _G
    assert C == 32 * _G and H * W == 64 * 1024 and H % 8 == 0 and W % 128 == 0
    assert _GEND[-1] == n_grp
    shp = (4 * n_grp, 2, 256, 8, 128)
    strips = B * C * H // 8
    xt = x.reshape(strips, 8, W // 128, 128).transpose(0, 2, 1, 3).reshape(shp)
    unit_bytes = 2 * 256 * 8 * 128 * x.dtype.itemsize
    out = pl.pallas_call(
        _kernel,
        in_specs=[pl.BlockSpec(memory_space=pl.ANY)] * 3,
        out_specs=pl.BlockSpec(memory_space=pl.ANY),
        out_shape=jax.ShapeDtypeStruct(shp, x.dtype),
        scratch_shapes=[
            pltpu.VMEM((4 * _S + 1,) + shp[1:], x.dtype),
            pltpu.VMEM((C,), g.dtype),
            pltpu.VMEM((C,), b.dtype),
            pltpu.VMEM((2 * C,), jnp.float32),
            pltpu.SMEM((2 * C,), jnp.float32),
            pltpu.SemaphoreType.DMA((4,)),
            pltpu.SemaphoreType.DMA((2,)),
        ],
        compiler_params=pltpu.CompilerParams(
            vmem_limit_bytes=(4 * _S + 1) * unit_bytes + 8 * 1024 * 1024),
    )(xt, g, b)
    return out.reshape(strips, W // 128, 8, 128).transpose(0, 2, 1, 3).reshape(x.shape)
```
